```python
import os as _os
_os.environ.setdefault("JAX_PLATFORMS", "cpu")
import jax
import jax.numpy as jnp

def _softmax(x, axis=-1):
    return jax.nn.softmax(x, axis=axis)
def _gelu(x):
    return jax.nn.gelu(x, approximate=True)
def _silu(x):
    return jax.nn.silu(x)
def _sigmoid(x):
    return jax.nn.sigmoid(x)
def _layernorm(x, axis=-1, eps=1e-5):
    m = jnp.mean(x, axis=axis, keepdims=True)
    v = jnp.var(x, axis=axis, keepdims=True)
    return (x - m) / jnp.sqrt(v + eps)
def _scatter_add(tgt, idx, src, axis=0):
    return tgt.at[idx].add(src)
def _segment_sum(src, seg, n):
    return jax.ops.segment_sum(src, seg, n)
class _Rng:
    def __init__(self, key):
        self._k = key
    def _next(self):
        self._k, sub = jax.random.split(self._k)
        return sub
    def normal(self, shape):
        return jax.random.normal(self._next(), shape, dtype=jnp.bfloat16)
    def randint(self, lo, hi, shape):
        return jax.random.randint(self._next(), shape, lo, hi, dtype=jnp.int32)
    def uniform(self, shape, lo=0.0, hi=1.0):
        return jax.random.uniform(self._next(), shape, jnp.bfloat16, lo, hi)
    def permutation(self, n):
        return jax.random.permutation(self._next(), n)


kernel_name = 'sequential_preLN__linear_kernel_hedgehog__glu_gated_swiglu__prompt'

def setup_inputs():
    _rng = _Rng(jax.random.key(int.from_bytes(__import__("os").urandom(4), "little")))
    _w = (lambda a: (lambda t: t.astype(jnp.bfloat16) if jnp.issubdtype(t.dtype, jnp.floating) else t)(jnp.asarray(a)))
    def _A_setup():
        B, S, D, H = 1, 2048, 640, 32
        Dh = D // H
        return {
            "x": _w((lambda *s: _rng.normal(s) * 0.05)(B, S, D)),
            "wqkv": _w((lambda *s: _rng.normal(s) * 0.2)(D, 3 * D)),
            "w_phi": _w((lambda *s: _rng.normal(s) * 0.2)(H, Dh, Dh) * (Dh ** -0.5)),
            "wo": _w((lambda *s: _rng.normal(s) * 0.05)(D, D)),
        }
    _A_in = _A_setup()

    def _B_setup():
        B, S, D, F = 1, 2048, 640, 1536
        return {
            "x": _w((lambda *s: _rng.normal(s) * 0.05)(B, S, D)),
            "w1": _w((lambda *s: _rng.normal(s) * 0.05)(D, F) * (2.0 / D) ** 0.5),
            "w3": _w((lambda *s: _rng.normal(s) * 0.05)(D, F) * (2.0 / D) ** 0.5),
            "w2": _w((lambda *s: _rng.normal(s) * 0.05)(F, D) * (2.0 / F) ** 0.5),
        }
    _B_in = _B_setup()

    return {
        "A_x": _A_in["x"],
        "A_wqkv": _A_in["wqkv"],
        "A_w_phi": _A_in["w_phi"],
        "A_wo": _A_in["wo"],
        "B_x": _B_in["x"],
        "B_w1": _B_in["w1"],
        "B_w3": _B_in["w3"],
        "B_w2": _B_in["w2"],
    }

def reference(A_x, A_wqkv, A_w_phi, A_wo, B_x, B_w1, B_w3, B_w2):
    def _A_ref(x, wqkv, w_phi, wo):
        B, S, D = x.shape
        H = 32; Dh = D // H
        qkv = (lambda x, *d: x.transpose(*d))((x @ wqkv).reshape(B, S, 3, H, Dh), 2, 0, 3, 1, 4)
        q, k, v = qkv[0], qkv[1], qkv[2]
        pq = jnp.einsum("bhsd,hdf->bhsf", q, w_phi)
        pk = jnp.einsum("bhsd,hdf->bhsf", k, w_phi)
        phi_q = jnp.concatenate([_softmax(pq, axis=-1), _softmax(-pq, axis=-1)], axis=-1)
        phi_k = jnp.concatenate([_softmax(pk, axis=-1), _softmax(-pk, axis=-1)], axis=-1)
        kv = jnp.einsum("bhsf,bhsd->bhfd", phi_k, v)
        z  = jnp.einsum("bhsf->bhf", phi_k)
        num = jnp.einsum("bhqf,bhfd->bhqd", phi_q, kv)
        den = jnp.einsum("bhqf,bhf->bhq", phi_q, z)[..., None] + 1e-6
        o = num / den
        return (lambda x, *d: x.transpose(*d))(o, 0, 2, 1, 3).reshape(B, S, D) @ wo

    def _B_ref(x, w1, w3, w2):
        gate = jnp.einsum("bsd,df->bsf", x, w1)
        up = jnp.einsum("bsd,df->bsf", x, w3)
        h = _silu(gate) * up
        out = jnp.einsum("bsf,fd->bsd", h, w2)
        return out

    x = A_x
    h = x + _A_ref(_layernorm(x, axis=-1), A_wqkv, A_w_phi, A_wo)
    h2 = h + _B_ref(_layernorm(h, axis=-1), B_w1, B_w3, B_w2)
    return h2
```

```python
import jax
import jax.numpy as jnp
from jax import lax
import jax.experimental.pallas as pl
import jax.experimental.pallas.tpu as pltpu

S, D, H, DH, F = 2048, 640, 32, 20, 1536
NG = H // 2
GW = 2 * DH
TS1 = 512
TS2 = 512
CH = 4
XV = 1
NB1 = S // TS1
NB2 = S // TS2
BF = jnp.bfloat16
F32 = jnp.float32
NT = (((1,), (1,)), ((), ()))
LOG2E = 1.4426950408889634


def _ln(x):
    m = jnp.mean(x, axis=-1, keepdims=True)
    xc = x - m
    v = jnp.mean(xc * xc, axis=-1, keepdims=True)
    return xc * lax.rsqrt(v + 1e-5)


def _allred(x, op):
    x = op(x, pltpu.roll(x, 2, 0))
    return op(x, pltpu.roll(x, 4, 0))


def _feature_map(p):
    t = p.shape[-1]
    p3 = p.reshape(GW // 8, 8, t)
    mx = _allred(jnp.max(p3, axis=0), jnp.maximum)
    mn = _allred(jnp.min(p3, axis=0), jnp.minimum)
    ep = jnp.exp2(p3 - mx[None])
    en = jnp.exp2(mn[None] - p3)
    rp = 1.0 / _allred(jnp.sum(ep, axis=0), jnp.add)
    rn = 1.0 / _allred(jnp.sum(en, axis=0), jnp.add)
    phi = jnp.concatenate([ep * rp[None], en * rn[None]], axis=0)
    return phi.reshape(2 * GW, t).astype(BF)


def _kernel(x_hbm, wqkv_hbm, wphi_hbm, wo_hbm, w1_hbm, w3_hbm, w2_hbm, out_hbm,
            x_v, wqkv_v, wphi_v, wo_v, w1_v, w3_v, w2_v, out_v,
            xn_v, wkv_v, wq_v, a_v, acc_v, kvt_v,
            sems, xsems, osems):
    cp_phi = pltpu.make_async_copy(wphi_hbm, wphi_v, sems.at[0])
    cp_k = pltpu.make_async_copy(wqkv_hbm.at[:, pl.ds(D, D)], wqkv_v.at[:, pl.ds(D, D)], sems.at[1])
    cp_v = pltpu.make_async_copy(wqkv_hbm.at[:, pl.ds(2 * D, D)], wqkv_v.at[:, pl.ds(2 * D, D)], sems.at[6])
    cp_q = pltpu.make_async_copy(wqkv_hbm.at[:, pl.ds(0, D)], wqkv_v.at[:, pl.ds(0, D)], sems.at[7])
    cp_wo = pltpu.make_async_copy(wo_hbm, wo_v, sems.at[2])
    cp_w1 = pltpu.make_async_copy(w1_hbm, w1_v, sems.at[3])
    cp_w3 = pltpu.make_async_copy(w3_hbm, w3_v, sems.at[4])
    cp_w2 = pltpu.make_async_copy(w2_hbm, w2_v, sems.at[5])

    def cp_x(i):
        return pltpu.make_async_copy(x_hbm.at[pl.ds(i * TS1, TS1)], x_v.at[pl.ds(i * TS1, TS1)], xsems.at[i])

    def cp_out(i):
        return pltpu.make_async_copy(out_v.at[pl.ds(i * TS2, TS2)], out_hbm.at[pl.ds(i * TS2, TS2)], osems.at[i])

    cp_phi.start()
    cp_k.start()
    cp_v.start()
    cp_x(0).start()

    acc_v[...] = jnp.zeros(acc_v.shape, F32)
    a_v[...] = jnp.zeros(a_v.shape, F32)
    j = lax.broadcasted_iota(jnp.int32, (D, D), 0)
    c = lax.broadcasted_iota(jnp.int32, (D, D), 1)
    perm = jnp.where(c == (j & 31) * DH + (j >> 5), 1.0, 0.0).astype(BF)
    r = lax.broadcasted_iota(jnp.int32, (GW, 32), 0)
    c = lax.broadcasted_iota(jnp.int32, (GW, 32), 1)
    esel = jnp.where(c == (r >> 1), 1.0, 0.0).astype(BF)
    cp_phi.wait()
    for d in range(DH):
        a_v[0:DH, 32 * d:32 * (d + 1)] = wphi_v[d].astype(F32)
    a2 = jnp.dot(a_v[...].astype(BF), perm, preferred_element_type=F32).astype(BF)
    t40 = jnp.dot(esel, a2, preferred_element_type=F32)
    r = lax.broadcasted_iota(jnp.int32, (GW, 128), 0)
    c = lax.broadcasted_iota(jnp.int32, (GW, 128), 1)
    pts = []
    for t in range(5):
        blocks = []
        for jj in range(4):
            lo = ((r & 1) + 2 * (3 * t + jj)) * DH - 128 * t
            blocks.append(jnp.where((c >= lo) & (c < lo + DH), t40[:, 128 * t:128 * (t + 1)], 0.0))
        pts.append(jnp.concatenate(blocks, axis=0).astype(BF))

    def fold(col0):
        rs = [lax.dot_general(pts[t], wqkv_v[:, col0 + 128 * t:col0 + 128 * (t + 1)], NT,
                              preferred_element_type=F32) for t in range(5)]
        parts = [rs[0][0:120]]
        for t in range(1, 5):
            parts.append(rs[t - 1][120:160] + rs[t][0:40])
            parts.append(rs[t][40:120])
        parts.append(rs[4][120:160])
        return (jnp.concatenate(parts, axis=0) * LOG2E).astype(BF)

    cw = CH * GW
    cp_k.wait()
    cp_q.start()
    for i in range(1, NB1):
        cp_x(i).start()
    wk = fold(D)
    for cc in range(NG // CH):
        wkv_v[2 * cw * cc:2 * cw * cc + cw, :] = wk[cw * cc:cw * (cc + 1)]
    cp_v.wait()
    if XV:
        wv = wqkv_v[:, 2 * D:3 * D].T
    else:
        r = lax.broadcasted_iota(jnp.int32, (128, 128), 0)
        c = lax.broadcasted_iota(jnp.int32, (128, 128), 1)
        eye = jnp.where(r == c, 1.0, 0.0).astype(BF)
        wv = jnp.concatenate([lax.dot_general(
            eye, wqkv_v[:, 2 * D + 128 * t:2 * D + 128 * (t + 1)], NT, preferred_element_type=F32).astype(BF)
            for t in range(5)], axis=0)
    for cc in range(NG // CH):
        wkv_v[2 * cw * cc + cw:2 * cw * (cc + 1), :] = wv[cw * cc:cw * (cc + 1)]
    cp_q.wait()
    cp_wo.start()
    cp_w1.start()
    cp_w3.start()
    cp_w2.start()
    wq_v[...] = fold(0)

    def phase1(i, carry):
        cp_x(i).wait()
        row0 = pl.multiple_of(i * TS1, TS1)
        xn = _ln(x_v[pl.ds(row0, TS1), :].astype(F32)).astype(BF)
        xn_v[pl.ds(row0, TS1), :] = xn
        ones = jnp.ones((8, TS1), F32)
        for cc in range(NG // CH):
            pr = lax.dot_general(wkv_v[2 * cw * cc:2 * cw * (cc + 1), :], xn, NT, preferred_element_type=F32)
            for jj in range(CH):
                g = cc * CH + jj
                phi = jnp.concatenate(
                    [_feature_map(pr[GW * jj:GW * (jj + 1), 128 * t:128 * (t + 1)]) for t in range(TS1 // 128)],
                    axis=1)
                vt = jnp.concatenate([pr[cw + GW * jj:cw + GW * (jj + 1)], ones], axis=0).astype(BF)
                acc_v[g] += lax.dot_general(vt, phi, NT, preferred_element_type=F32)
        return carry

    lax.fori_loop(0, NB1, phase1, 0)

    r = lax.broadcasted_iota(jnp.int32, (GW + 8, 2 * GW), 0)
    c = lax.broadcasted_iota(jnp.int32, (GW + 8, 2 * GW), 1)
    hh = jnp.where(r < GW, jnp.where(r >= DH, 1, 0), jnp.where(r >= GW + 4, 1, 0))
    msk = hh == (c & 1)
    for g in range(NG):
        kvt_v[g] = jnp.where(msk, acc_v[g], 0.0).astype(BF)
    cp_wo.wait()
    cp_w1.wait()
    cp_w3.wait()
    cp_w2.wait()

    def phase2(i, carry):
        row0 = pl.multiple_of(i * TS2, TS2)
        xn = xn_v[pl.ds(row0, TS2), :]
        low = lax.broadcasted_iota(jnp.int32, (8, TS2), 0) < 4
        cq = 2 * cw if 2 * cw <= D else cw
        ots = []
        for cc in range(D // cq):
            pr = lax.dot_general(wq_v[cq * cc:cq * (cc + 1), :], xn, NT, preferred_element_type=F32)
            for jj in range(cq // GW):
                g = cc * (cq // GW) + jj
                phi = jnp.concatenate(
                    [_feature_map(pr[GW * jj:GW * (jj + 1), 128 * t:128 * (t + 1)]) for t in range(TS2 // 128)],
                    axis=1)
                nd = jnp.dot(kvt_v[g], phi, preferred_element_type=F32)
                rd = 1.0 / (nd[GW:GW + 8] + 1e-6)
                rs = pltpu.roll(rd, 4, 0)
                r0 = jnp.where(low, rd, rs)
                r1 = jnp.where(low, rs, rd)
                ots += [nd[0:8] * r0, nd[8:16] * r0, nd[16:24] * rd, nd[24:32] * r1, nd[32:40] * r1]
        o = jnp.concatenate(ots, axis=0).T.astype(BF)
        h = x_v[pl.ds(row0, TS2), :].astype(F32) + jnp.dot(o, wo_v[...], preferred_element_type=F32)
        hn = _ln(h).astype(BF)
        gate = jnp.dot(hn, w1_v[...], preferred_element_type=F32)
        up = jnp.dot(hn, w3_v[...], preferred_element_type=F32)
        act = (gate * up / (1.0 + jnp.exp(-gate))).astype(BF)
        out_v[pl.ds(row0, TS2), :] = (h + jnp.dot(act, w2_v[...], preferred_element_type=F32)).astype(BF)
        cp_out(i).start()
        return carry

    lax.fori_loop(0, NB2, phase2, 0)
    for i in range(NB2):
        cp_out(i).wait()


@jax.jit
def pallas_sequential_preLN__linear_kernel_hedgehog__glu_gated_swiglu__prompt_kernel(
    A_x, A_wqkv, A_w_phi, A_wo, B_x, B_w1, B_w3, B_w2,
):
    del B_x
    anyspec = pl.BlockSpec(memory_space=pl.ANY)
    out = pl.pallas_call(
        _kernel,
        in_specs=[anyspec] * 7,
        out_specs=anyspec,
        out_shape=jax.ShapeDtypeStruct((S, D), BF),
        scratch_shapes=[
            pltpu.VMEM((S, D), BF),
            pltpu.VMEM((D, 3 * D), BF),
            pltpu.VMEM((DH, DH, H), BF),
            pltpu.VMEM((D, D), BF),
            pltpu.VMEM((D, F), BF),
            pltpu.VMEM((D, F), BF),
            pltpu.VMEM((F, D), BF),
            pltpu.VMEM((S, D), BF),
            pltpu.VMEM((S, D), BF),
            pltpu.VMEM((2 * D, D), BF),
            pltpu.VMEM((D, D), BF),
            pltpu.VMEM((32, D), F32),
            pltpu.VMEM((NG, GW + 8, 2 * GW), F32),
            pltpu.VMEM((NG, GW + 8, 2 * GW), BF),
            pltpu.SemaphoreType.DMA((8,)),
            pltpu.SemaphoreType.DMA((NB1,)),
            pltpu.SemaphoreType.DMA((NB2,)),
        ],
        compiler_params=pltpu.CompilerParams(vmem_limit_bytes=100 * 1024 * 1024),
    )(A_x.reshape(S, D), A_wqkv, jnp.transpose(A_w_phi, (1, 2, 0)), A_wo, B_w1, B_w3, B_w2)
    return out.reshape(1, S, D)
```

```python
import jax
import jax.numpy as jnp
from jax import lax
import jax.experimental.pallas as pl
import jax.experimental.pallas.tpu as pltpu

S, D, H, DH, F = 2048, 640, 32, 20, 1536
NG = H // 2
GW = 2 * DH
TS = 512
NB = S // TS
CH = 8
CH0 = 4
CQ = 8
KA = 384
SC = 0
HS = 2
LN = 0
ORD = 3
UW = 512
BF = jnp.bfloat16
F32 = jnp.float32
NT = (((1,), (1,)), ((), ()))
LOG2E = 1.4426950408889634


def _wait(cp, name):
    if SC:
        with jax.named_scope(name):
            cp.wait()
    else:
        cp.wait()


def _ln(x):
    if LN == 0:
        m = jnp.mean(x, axis=-1, keepdims=True)
        xc = x - m
        v = jnp.mean(xc * xc, axis=-1, keepdims=True)
        return xc * lax.rsqrt(v + 1e-5)
    if LN == 1:
        x0 = x[:, 0:1]
        d = x - x0
        m = jnp.sum(d, axis=-1, keepdims=True) * (1.0 / D)
        v = jnp.sum(d * d, axis=-1, keepdims=True) * (1.0 / D) - m * m
        return (x - (x0 + m)) * lax.rsqrt(jnp.maximum(v, 0.0) + 1e-5)
    m = jnp.sum(x, axis=-1, keepdims=True) * (1.0 / D)
    v = jnp.sum(x * x, axis=-1, keepdims=True) * (1.0 / D) - m * m
    return (x - m) * lax.rsqrt(jnp.maximum(v, 0.0) + 1e-5)


def _allred(x, op):
    x = op(x, pltpu.roll(x, 2, 0))
    return op(x, pltpu.roll(x, 4, 0))


def _feature_map1(p):
    t = p.shape[-1]
    p3 = p.reshape(GW // 8, 8, t)
    mx = _allred(jnp.max(p3, axis=0), jnp.maximum)
    mn = _allred(jnp.min(p3, axis=0), jnp.minimum)
    ep = jnp.exp2(p3 - mx[None])
    en = jnp.exp2(mn[None] - p3)
    rp = 1.0 / _allred(jnp.sum(ep, axis=0), jnp.add)
    rn = 1.0 / _allred(jnp.sum(en, axis=0), jnp.add)
    phi = jnp.concatenate([ep * rp[None], en * rn[None]], axis=0)
    return phi.reshape(2 * GW, t).astype(BF)


def _feature_map(p):
    return jnp.concatenate(
        [_feature_map1(p[:, 128 * t:128 * (t + 1)]) for t in range(p.shape[-1] // 128)], axis=1)


def _kernel(x_hbm, wqkv_hbm, wphi_hbm, wo_hbm, w1_hbm, w3_hbm, w2_hbm, out_hbm,
            x_v, wqkv_v, wphi_v, wo_v, w1_v, w3_v, w2_v, out_v,
            xn_v, wkv_v, wq_v, a_v, kvt_v,
            sems, osems):
    def cp_w(r0, nr, c0, s):
        return pltpu.make_async_copy(wqkv_hbm.at[pl.ds(r0, nr), pl.ds(c0, D)],
                                     wqkv_v.at[pl.ds(r0, nr), pl.ds(c0, D)], sems.at[s])

    def cp_x(r0, nr, s):
        return pltpu.make_async_copy(x_hbm.at[pl.ds(r0, nr)], x_v.at[pl.ds(r0, nr)], sems.at[s])

    cp_phi = pltpu.make_async_copy(wphi_hbm, wphi_v, sems.at[0])
    cp_ka = cp_w(0, KA, D, 1)
    cp_kb = cp_w(KA, D - KA, D, 2)
    cp_x0a = cp_x(0, TS // 2, 3)
    cp_x0b = cp_x(TS // 2, TS // 2, 4)
    cp_v = cp_w(0, D, 2 * D, 5)
    cp_xs = [cp_x(TS * i, TS, 5 + i) for i in range(1, NB)]
    cp_q = cp_w(0, D, 0, 9)
    cp_wo = pltpu.make_async_copy(wo_hbm, wo_v, sems.at[10])
    cp_w1 = pltpu.make_async_copy(w1_hbm, w1_v, sems.at[11])
    cp_w3 = pltpu.make_async_copy(w3_hbm, w3_v, sems.at[12])
    cp_w2 = pltpu.make_async_copy(w2_hbm, w2_v, sems.at[13])
    for cp in [cp_phi, cp_ka, cp_kb, cp_x0a, cp_x0b, cp_xs[0], cp_v, cp_xs[1], cp_xs[2], cp_q, cp_wo, cp_w1, cp_w3, cp_w2]:
        cp.start()

    a_v[...] = jnp.zeros(a_v.shape, F32)
    j = lax.broadcasted_iota(jnp.int32, (D, D), 0)
    c = lax.broadcasted_iota(jnp.int32, (D, D), 1)
    perm = jnp.where(c == (j & 31) * DH + (j >> 5), 1.0, 0.0).astype(BF)
    r = lax.broadcasted_iota(jnp.int32, (GW, 32), 0)
    c = lax.broadcasted_iota(jnp.int32, (GW, 32), 1)
    esel = jnp.where(c == (r >> 1), 1.0, 0.0).astype(BF)
    _wait(cp_phi, 'w_phi')
    for d in range(DH):
        a_v[0:DH, 32 * d:32 * (d + 1)] = wphi_v[d].astype(F32)
    a2 = jnp.dot(a_v[...].astype(BF), perm, preferred_element_type=F32).astype(BF)
    t40 = jnp.dot(esel, a2, preferred_element_type=F32)
    r = lax.broadcasted_iota(jnp.int32, (GW, 128), 0)
    c = lax.broadcasted_iota(jnp.int32, (GW, 128), 1)
    pts = []
    for t in range(5):
        blocks = []
        for jj in range(4):
            lo = ((r & 1) + 2 * (3 * t + jj)) * DH - 128 * t
            blocks.append(jnp.where((c >= lo) & (c < lo + DH), t40[:, 128 * t:128 * (t + 1)], 0.0))
        pts.append(jnp.concatenate(blocks, axis=0).astype(BF))

    def fold(col0, r0, r1):
        rs = [lax.dot_general(pts[t], wqkv_v[r0:r1, col0 + 128 * t:col0 + 128 * (t + 1)], NT,
                              preferred_element_type=F32) for t in range(5)]
        parts = [rs[0][0:120]]
        for t in range(1, 5):
            parts.append(rs[t - 1][120:160] + rs[t][0:40])
            parts.append(rs[t][40:120])
        parts.append(rs[4][120:160])
        return (jnp.concatenate(parts, axis=0) * LOG2E).astype(BF)

    def norm(r0, nr):
        xn = _ln(x_v[r0:r0 + nr, :].astype(F32)).astype(BF)
        xn_v[r0:r0 + nr, :] = xn
        return xn

    def proj(w_v, g0, ng, xn):
        return lax.dot_general(w_v[GW * g0:GW * (g0 + ng), :], xn, NT, preferred_element_type=F32)

    def kv_update(acc, g, v, phi):
        vt = jnp.concatenate([v, jnp.ones((8, v.shape[1]), F32)], axis=0).astype(BF)
        u = lax.dot_general(vt, phi, NT, preferred_element_type=F32)
        acc[g] = u if acc[g] is None else acc[g] + u

    _wait(cp_ka, 'w_ka')
    wkv_v[0:D, 0:KA] = fold(D, 0, KA)
    _wait(cp_kb, 'w_kb')
    wkv_v[0:D, KA:D] = fold(D, KA, D)

    acc = [None] * NG
    xns, pks, pvs, phis = {}, {}, {}, {}
    C4 = 4

    def L(tb, r0, nr):
        xns[tb] = norm(r0, nr)

    def K(tb, c0, c1):
        p = proj(wkv_v, C4 * c0, C4 * (c1 - c0), xns[tb])
        for g in range(C4 * c0, C4 * c1):
            pks[tb, g] = p[GW * (g - C4 * c0):GW * (g - C4 * c0 + 1)]

    def V(tb, c0, c1):
        p = proj(wkv_v, NG + C4 * c0, C4 * (c1 - c0), xns[tb])
        for g in range(C4 * c0, C4 * c1):
            pvs[tb, g] = p[GW * (g - C4 * c0):GW * (g - C4 * c0 + 1)]

    def Fm(tb, c0, c1):
        for g in range(C4 * c0, C4 * c1):
            phis[tb, g] = _feature_map(pks[tb, g])

    def KV(tb, c0, c1):
        for g in range(C4 * c0, C4 * c1):
            phi = jnp.concatenate([phis['a', g], phis['b', g]], axis=1) if tb == 0 else phis[tb, g]
            kv_update(acc, g, pvs[tb, g], phi)

    _wait(cp_x0a, 'w_x0a')
    L('a', 0, TS // 2)
    K('a', 0, 2)
    _wait(cp_x0b, 'w_x0b')
    L('b', TS // 2, TS // 2)
    xns[0] = jnp.concatenate([xns['a'], xns['b']], axis=0)
    Fm('a', 0, 2)
    K('a', 2, 4)
    Fm('a', 2, 3)
    K('b', 0, 2)
    K('b', 2, 3)
    _wait(cp_xs[0], 'w_x1')
    _wait(cp_v, 'w_v')
    L(1, TS, TS)
    wkv_v[D:2 * D, :] = wqkv_v[:, 2 * D:3 * D].T
    K('b', 3, 4)
    Fm('a', 3, 4)
    Fm('b', 0, 4)
    K(1, 0, 2)
    K(1, 2, 4)
    V(0, 0, 2)
    Fm(1, 0, 2)
    KV(0, 0, 2)
    V(0, 2, 4)
    KV(0, 2, 4)
    V(1, 0, 2)
    Fm(1, 2, 4)
    KV(1, 0, 2)
    _wait(cp_xs[1], 'w_x2')
    _wait(cp_xs[2], 'w_x3')
    _wait(cp_q, 'w_q')
    if ORD < 3:
        L(2, 2 * TS, TS)
    V(1, 2, 4)
    KV(1, 2, 4)
    if ORD == 0:
        for i in range(2, NB):
            for c in (0, 2):
                K(i, c, c + 2)
                Fm(i, c, c + 2)
                if c == 2 and i + 1 < NB:
                    L(i + 1, TS * (i + 1), TS)
                V(i, c, c + 2)
                KV(i, c, c + 2)
    elif ORD == 1:
        prev = None
        for i in range(2, NB):
            for c in range(4):
                K(i, c, c + 1)
                Fm(i, c, c + 1)
                if c == 2 and i + 1 < NB:
                    L(i + 1, TS * (i + 1), TS)
                V(i, c, c + 1)
                if prev is not None:
                    KV(*prev)
                prev = (i, c, c + 1)
        KV(*prev)
    elif ORD == 2:
        for i in range(2, NB):
            K(i, 0, 4)
            Fm(i, 0, 4)
            if i + 1 < NB:
                L(i + 1, TS * (i + 1), TS)
            V(i, 0, 4)
            KV(i, 0, 4)
    else:
        for u in range(2 * TS // UW):
            tb = ('u', u)
            L(tb, 2 * TS + UW * u, UW)
            p = proj(wkv_v, 0, 2 * NG, xns[tb])
            for g in range(NG):
                kv_update(acc, g, p[D + GW * g:D + GW * (g + 1)], _feature_map(p[GW * g:GW * (g + 1)]))

    wq_v[...] = fold(0, 0, D)

    r = lax.broadcasted_iota(jnp.int32, (GW + 8, 2 * GW), 0)
    c = lax.broadcasted_iota(jnp.int32, (GW + 8, 2 * GW), 1)
    hh = jnp.where(r < GW, jnp.where(r >= DH, 1, 0), jnp.where(r >= GW + 4, 1, 0))
    msk = hh == (c & 1)
    for g in range(NG):
        kvt_v[g] = jnp.where(msk, acc[g], 0.0).astype(BF)
    _wait(cp_wo, 'w_wo')
    cp_w1.wait()
    cp_w3.wait()
    cp_w2.wait()

    hs = TS // HS
    pieces = [(hs * p, hs) for p in range(HS - 1)] + [(TS - hs, hs // 2), (TS - hs // 2, hs // 2)]

    def cp_out(i, p):
        r0 = pl.multiple_of(i * TS + pieces[p][0], 128)
        return pltpu.make_async_copy(out_v.at[pl.ds(r0, pieces[p][1])], out_hbm.at[pl.ds(r0, pieces[p][1])],
                                     osems.at[i, p])

    def phase2(i, carry):
        row0 = pl.multiple_of(i * TS, TS)
        xn = xn_v[pl.ds(row0, TS), :]
        low = lax.broadcasted_iota(jnp.int32, (8, TS), 0) < 4
        ots = []
        for cc in range(NG // CQ):
            pr = proj(wq_v, CQ * cc, CQ, xn)
            for jj in range(CQ):
                g = cc * CQ + jj
                phi = _feature_map(pr[GW * jj:GW * (jj + 1)])
                nd = jnp.dot(kvt_v[g], phi, preferred_element_type=F32)
                rd = 1.0 / (nd[GW:GW + 8] + 1e-6)
                rs = pltpu.roll(rd, 4, 0)
                r0 = jnp.where(low, rd, rs)
                r1 = jnp.where(low, rs, rd)
                ots += [nd[0:8] * r0, nd[8:16] * r0, nd[16:24] * rd, nd[24:32] * r1, nd[32:40] * r1]
        ot = jnp.concatenate(ots, axis=0)
        hsv = []
        for p in range(HS):
            o = ot[:, hs * p:hs * (p + 1)].T.astype(BF)
            rp = pl.multiple_of(row0 + hs * p, hs)
            hsv.append(x_v[pl.ds(rp, hs), :].astype(F32) + jnp.dot(o, wo_v[...], preferred_element_type=F32))
        acts = []
        for p in range(HS):
            hn = _ln(hsv[p]).astype(BF)
            gate = jnp.dot(hn, w1_v[...], preferred_element_type=F32)
            up = jnp.dot(hn, w3_v[...], preferred_element_type=F32)
            acts.append((gate * up / (1.0 + jnp.exp(-gate))).astype(BF))
        for p, (r0, nr) in enumerate(pieces):
            hp, off = divmod(r0, hs)
            y = hsv[hp][off:off + nr] + jnp.dot(acts[hp][off:off + nr], w2_v[...], preferred_element_type=F32)
            out_v[pl.ds(pl.multiple_of(row0 + r0, 128), nr), :] = y.astype(BF)
            cp_out(i, p).start()
        return carry

    lax.fori_loop(0, NB, phase2, 0)
    for i in range(NB):
        for p in range(len(pieces)):
            _wait(cp_out(i, p), 'w_out')


@jax.jit
def pallas_sequential_preLN__linear_kernel_hedgehog__glu_gated_swiglu__prompt_kernel(
    A_x, A_wqkv, A_w_phi, A_wo, B_x, B_w1, B_w3, B_w2,
):
    del B_x
    anyspec = pl.BlockSpec(memory_space=pl.ANY)
    out = pl.pallas_call(
        _kernel,
        in_specs=[anyspec] * 7,
        out_specs=anyspec,
        out_shape=jax.ShapeDtypeStruct((S, D), BF),
        scratch_shapes=[
            pltpu.VMEM((S, D), BF),
            pltpu.VMEM((D, 3 * D), BF),
            pltpu.VMEM((DH, DH, H), BF),
            pltpu.VMEM((D, D), BF),
            pltpu.VMEM((D, F), BF),
            pltpu.VMEM((D, F), BF),
            pltpu.VMEM((F, D), BF),
            pltpu.VMEM((S, D), BF),
            pltpu.VMEM((S, D), BF),
            pltpu.VMEM((2 * D, D), BF),
            pltpu.VMEM((D, D), BF),
            pltpu.VMEM((32, D), F32),
            pltpu.VMEM((NG, GW + 8, 2 * GW), BF),
            pltpu.SemaphoreType.DMA((14,)),
            pltpu.SemaphoreType.DMA((NB, HS + 1)),
        ],
        compiler_params=pltpu.CompilerParams(vmem_limit_bytes=100 * 1024 * 1024),
    )(A_x.reshape(S, D), A_wqkv, jnp.transpose(A_w_phi, (1, 2, 0)), A_wo, B_w1, B_w3, B_w2)
    return out.reshape(1, S, D)
```

```python
import jax
import jax.numpy as jnp
from jax import lax
import jax.experimental.pallas as pl
import jax.experimental.pallas.tpu as pltpu

S, D, H, DH, F = 2048, 640, 32, 20, 1536
NG = H // 2
GW = 2 * DH
TS = 512
NB = S // TS
HR = TS // 2
KP = (3, 2)
XP = (256, 256, 256, 640, 640)
DMA_ORDER = ('phi', 'k0', 'x0', 'k1', 'x1', 'v', 'x2', 'x3', 'x4', 'q', 'wo', 'w1', 'w3', 'w2')
PIECES = ((0, 0, D), (HR, 0, 256), (HR, 256, 256), (HR, 512, 128))
BF = jnp.bfloat16
F32 = jnp.float32
NT = (((1,), (1,)), ((), ()))
LOG2E = 1.4426950408889634


def _recip(x):
    r = pl.reciprocal(x, approx=True)
    return r * (2.0 - x * r)


def _swiglu(g, u):
    return g * u * _recip(1.0 + jnp.exp(jnp.minimum(-g, 80.0)))


def _zero(g):
    u = lax.bitcast_convert_type(g, jnp.uint32)
    u = lax.shift_right_logical(lax.shift_right_logical(u, jnp.uint32(16)), jnp.uint32(16))
    return lax.bitcast_convert_type(u, F32)


def _lanesum(x):
    s = x[:, 0:128]
    for t in range(1, x.shape[1] // 128):
        s = s + x[:, 128 * t:128 * (t + 1)]
    return s


def _layernorm(x, toks):
    n = x.shape[0] // len(toks)
    outs = []
    for j, tok in enumerate(toks):
        xj = x[n * j:n * (j + 1)]
        s = _lanesum(xj) + jnp.concatenate([_zero(tok)] * (n // 8), axis=0)
        xc = xj - jnp.sum(s, axis=-1, keepdims=True) * (1.0 / D)
        v = jnp.mean(xc * xc, axis=-1, keepdims=True)
        outs.append(xc * lax.rsqrt(v + 1e-5))
    return jnp.concatenate(outs, axis=0)


def _stats(x):
    s1 = jnp.sum(_lanesum(x).T.reshape(16, 8, 128), axis=0)
    s2 = jnp.sum(_lanesum(x * x).T.reshape(16, 8, 128), axis=0)
    for sh in (1, 2, 4):
        s1 = s1 + pltpu.roll(s1, sh, 0)
        s2 = s2 + pltpu.roll(s2, sh, 0)
    m = s1 * (1.0 / D)
    v = jnp.maximum(s2 * (1.0 / D) - m * m, 0.0)
    return m, lax.rsqrt(v + 1e-5)


def _allred(x, op):
    x = op(x, pltpu.roll(x, 2, 0))
    return op(x, pltpu.roll(x, 4, 0))


def _feature_map(p, sc):
    p3 = p.reshape(GW // 8, 8, 128) * sc[None]
    mx = _allred(jnp.max(p3, axis=0), jnp.maximum)
    mn = _allred(jnp.min(p3, axis=0), jnp.minimum)
    ep = jnp.exp2(p3 - mx[None])
    en = jnp.exp2(mn[None] - p3)
    rp = _recip(_allred(jnp.sum(ep, axis=0), jnp.add))
    rn = _recip(_allred(jnp.sum(en, axis=0), jnp.add))
    return jnp.concatenate([ep * rp[None], en * rn[None]], axis=0).reshape(2 * GW, 128)


def _kernel(x_hbm, wqkv_hbm, wphi_hbm, wo_hbm, w1_hbm, w3_hbm, w2_hbm, out_hbm,
            x_v, wqkv_v, wphi_v, wo_v, w1_v, w3_v, w2_v, out_v,
            rl_v, wkv_v, wq_v, a_v, kvt_v,
            sems, osems):
    def cp_w(c0, nc, s):
        return pltpu.make_async_copy(wqkv_hbm.at[:, pl.ds(c0, nc)], wqkv_v.at[:, pl.ds(c0, nc)], sems.at[s])

    cps = {'phi': pltpu.make_async_copy(wphi_hbm, wphi_v, sems.at[0])}
    for i, n in enumerate(KP):
        cps['k%d' % i] = cp_w(D + 128 * sum(KP[:i]), 128 * n, 1 + i)
    for i, n in enumerate(XP):
        rows = pl.ds(sum(XP[:i]), n)
        cps['x%d' % i] = pltpu.make_async_copy(x_hbm.at[rows], x_v.at[rows], sems.at[3 + i])
    cps['v'] = cp_w(2 * D, D, 8)
    cps['q'] = cp_w(0, D, 9)
    cps['wo'] = pltpu.make_async_copy(wo_hbm, wo_v, sems.at[10])
    cps['w1'] = pltpu.make_async_copy(w1_hbm, w1_v, sems.at[11])
    cps['w3'] = pltpu.make_async_copy(w3_hbm, w3_v, sems.at[12])
    cps['w2'] = pltpu.make_async_copy(w2_hbm, w2_v, sems.at[13])
    for name in DMA_ORDER:
        cps[name].start()

    def wait(*names):
        for name in names:
            cps[name].wait()

    a_v[...] = jnp.zeros(a_v.shape, F32)
    j = lax.broadcasted_iota(jnp.int32, (D, D), 0)
    c = lax.broadcasted_iota(jnp.int32, (D, D), 1)
    perm = jnp.where(c == (j & 31) * DH + (j >> 5), 1.0, 0.0).astype(BF)
    r = lax.broadcasted_iota(jnp.int32, (GW, 32), 0)
    c = lax.broadcasted_iota(jnp.int32, (GW, 32), 1)
    esel = jnp.where(c == (r >> 1), 1.0, 0.0).astype(BF)
    wait('phi')
    for d in range(DH):
        a_v[0:DH, 32 * d:32 * (d + 1)] = wphi_v[d].astype(F32)
    a2 = jnp.dot(a_v[...].astype(BF), perm, preferred_element_type=F32).astype(BF)
    t40 = jnp.dot(esel, a2, preferred_element_type=F32)
    r = lax.broadcasted_iota(jnp.int32, (GW, 128), 0)
    c = lax.broadcasted_iota(jnp.int32, (GW, 128), 1)
    pts = []
    for t in range(5):
        blocks = []
        for jj in range(4):
            lo = ((r & 1) + 2 * (3 * t + jj)) * DH - 128 * t
            blocks.append(jnp.where((c >= lo) & (c < lo + DH), t40[:, 128 * t:128 * (t + 1)], 0.0))
        pts.append(jnp.concatenate(blocks, axis=0).astype(BF))

    def fold(dst, col0, t0, t1, state):
        row, done, carry = state
        for t in range(t0, t1):
            rt = lax.dot_general(pts[t], wqkv_v[:, col0 + 128 * t:col0 + 128 * (t + 1)], NT,
                                 preferred_element_type=F32)
            done = done + [rt[0:GW] if carry is None else rt[0:GW] + carry, rt[GW:160 if t == 4 else 120]]
            carry = rt[120:160]
        w = jnp.concatenate(done, axis=0)
        n = w.shape[0] // 80 * 80
        wn = w[0:n]
        dst[row:row + n, :] = (wn - jnp.sum(_lanesum(wn), axis=-1, keepdims=True) * (1.0 / D)).astype(BF)
        return row + n, [w[n:]] if n < w.shape[0] else [], carry

    def proj(w_v, g0, ng, x):
        return lax.dot_general(w_v[GW * g0:GW * (g0 + ng), :], x, NT, preferred_element_type=F32)

    acc = [None] * NG
    pks, pvs, phis, rs, rls, exs = {}, {}, {}, {}, {}, {}
    low8 = lax.broadcasted_iota(jnp.int32, (8, 128), 0) < 4

    def stats(t0, t1):
        for t in range(t0, t1):
            m, rs[t] = _stats(x_v[128 * t:128 * (t + 1), :].astype(F32))
            exs[t] = jnp.where(low8, 1.0, m * rs[t])
            rls[t] = rs[t] * LOG2E
            rl_v[t] = rls[t]

    def kv_proj(dst, base, t0, t1, g0, g1):
        p = proj(wkv_v, base + g0, g1 - g0, x_v[128 * t0:128 * t1, :])
        for g in range(g0, g1):
            for t in range(t0, t1):
                dst[t, g] = p[GW * (g - g0):GW * (g - g0 + 1), 128 * (t - t0):128 * (t - t0 + 1)]

    def kproj(t0, t1, g0=0, g1=NG):
        kv_proj(pks, 0, t0, t1, g0, g1)

    def vproj(t0, t1, g0=0, g1=NG):
        kv_proj(pvs, NG, t0, t1, g0, g1)

    def feat(t0, t1, g0=0, g1=NG):
        for t in range(t0, t1):
            for g in range(g0, g1):
                phis[t, g] = _feature_map(pks[t, g], rls[t])

    def accum(t0, t1, g0=0, g1=NG):
        ts = range(t0, t1)
        for g in range(g0, g1):
            phi = jnp.concatenate([phis[t, g] for t in ts], axis=1).astype(BF)
            v = jnp.concatenate([(pvs[t, g].reshape(GW // 8, 8, 128) * rs[t][None]).reshape(GW, 128) for t in ts],
                                axis=1)
            vt = jnp.concatenate([v, jnp.concatenate([exs[t] for t in ts], axis=1)], axis=0).astype(BF)
            u = lax.dot_general(vt, phi, NT, preferred_element_type=F32)
            acc[g] = u if acc[g] is None else u + acc[g]

    wait('k0')
    fk = fold(wkv_v, D, 0, KP[0], (0, [], None))
    wait('x0')
    stats(0, 2)
    kproj(0, 2, 0, 4)
    feat(0, 2, 0, 4)
    kproj(0, 2, 4, 8)
    wait('k1', 'x1')
    fold(wkv_v, D, KP[0], 5, fk)
    stats(2, 4)
    kproj(2, 4, 0, 8)
    feat(0, 2, 4, 8)
    kproj(0, 4, 8, 12)
    wait('v', 'x2')
    wkv_v[D:2 * D, :] = wqkv_v[:, 2 * D:3 * D].T
    stats(4, 6)
    kproj(0, 4, 12, 16)
    feat(0, 4, 12, 16)
    vproj(0, 4, 12, 16)
    vproj(0, 4, 0, 4)
    feat(2, 4, 0, 4)
    vproj(0, 4, 4, 8)
    feat(2, 4, 4, 8)
    vproj(0, 4, 8, 12)
    feat(0, 4, 8, 12)
    kproj(4, 6, 0, 8)
    kproj(4, 6, 8, 16)
    wait('x3', 'x4', 'q')
    wv_sum = jnp.sum(_lanesum(wkv_v[D:2 * D, :].astype(F32)), axis=-1, keepdims=True)
    stats(6, 8)
    kproj(6, 8)
    feat(4, 8)
    for t in (4, 8, 12):
        if t > 4:
            kproj(t, t + 4)
            feat(t, t + 4)
        if t < 12:
            stats(t + 4, t + 8)
        for g in range(0, NG, 4):
            vproj(t, t + 4, g, g + 4)
            accum(t - 4, t, g, g + 4)
    accum(12, 16, 0, 8)
    fold(wq_v, 0, 0, 5, (0, [], None))
    accum(12, 16, 8, 16)

    r = lax.broadcasted_iota(jnp.int32, (GW + 8, 2 * GW), 0)
    c = lax.broadcasted_iota(jnp.int32, (GW + 8, 2 * GW), 1)
    hh = jnp.where(r < GW, jnp.where(r >= DH, 1, 0), jnp.where(r >= GW + 4, 1, 0))
    msk = hh == (c & 1)
    low80 = lax.broadcasted_iota(jnp.int32, (8, 2 * GW), 0) < 4
    for g in range(NG):
        tail = acc[g][GW:GW + 8]
        rot = pltpu.roll(tail, 4, 0)
        zt = jnp.where(low80, tail, rot)
        mt = jnp.where(low80, rot, tail)
        kv = acc[g][0:GW].reshape(GW // 8, 8, 2 * GW) - wv_sum[GW * g:GW * (g + 1)].reshape(GW // 8, 8, 1) * mt[None]
        kvt_v[g] = jnp.where(msk, jnp.concatenate([kv.reshape(GW, 2 * GW), zt], axis=0), 0.0).astype(BF)
    wait('wo', 'w1', 'w3', 'w2')

    def cp_out(i, p):
        r0, c0, nc = PIECES[p]
        rows = pl.ds(pl.multiple_of(i * TS + r0, HR), HR)
        return pltpu.make_async_copy(out_v.at[rows, pl.ds(c0, nc)], out_hbm.at[rows, pl.ds(c0, nc)], osems.at[i, p])

    def phase2(i, carry):
        row0 = pl.multiple_of(i * TS, TS)
        scs = [rl_v[(TS // 128) * i + t] for t in range(TS // 128)]
        low = lax.broadcasted_iota(jnp.int32, (8, TS), 0) < 4
        pq = proj(wq_v, 0, NG, x_v[pl.ds(row0, TS), :])
        ots = []
        for g in range(NG):
            phi = jnp.concatenate(
                [_feature_map(pq[GW * g:GW * (g + 1), 128 * t:128 * (t + 1)], scs[t]) for t in range(TS // 128)],
                axis=1).astype(BF)
            nd = jnp.dot(kvt_v[g], phi, preferred_element_type=F32)
            rd = _recip(nd[GW:GW + 8] + 1e-6)
            rr = pltpu.roll(rd, 4, 0)
            ra = jnp.where(low, rd, rr)
            rb = jnp.where(low, rr, rd)
            ots += [nd[0:8] * ra, nd[8:16] * ra, nd[16:24] * rd, nd[24:32] * rb, nd[32:40] * rb]
        ot = jnp.concatenate(ots, axis=0)
        hs, atts, acts = [], [], []
        for p in range(2):
            o = ot[:, HR * p:HR * (p + 1)].T.astype(BF)
            atts.append(jnp.dot(o, wo_v[...], preferred_element_type=F32))
            hs.append(x_v[pl.ds(pl.multiple_of(row0 + HR * p, HR), HR), :].astype(F32) + atts[-1])
        toks = [atts[1][HR - 8:HR, 128 * t:128 * (t + 1)] for t in range(4)]
        for p in range(2):
            hn = _layernorm(hs[p], toks).astype(BF)
            gate = jnp.dot(hn, w1_v[...], preferred_element_type=F32)
            up = jnp.dot(hn, w3_v[...], preferred_element_type=F32)
            acts.append(_swiglu(gate, up))
            toks = [gate[HR - 8:HR, 128 * t:128 * (t + 1)] for t in range(8)]
        actb = {}
        for p, (r0, c0, nc) in enumerate(PIECES):
            hp = r0 // HR
            if hp not in actb:
                actb[hp] = acts[hp].astype(BF)
            y = hs[hp][:, c0:c0 + nc] + jnp.dot(actb[hp], w2_v[:, c0:c0 + nc], preferred_element_type=F32)
            out_v[pl.ds(pl.multiple_of(row0 + r0, HR), HR), c0:c0 + nc] = y.astype(BF)
            cp_out(i, p).start()
        return carry

    lax.fori_loop(0, NB, phase2, 0)
    for i in range(NB):
        for p in range(len(PIECES)):
            cp_out(i, p).wait()


@jax.jit
def pallas_sequential_preLN__linear_kernel_hedgehog__glu_gated_swiglu__prompt_kernel(
    A_x, A_wqkv, A_w_phi, A_wo, B_x, B_w1, B_w3, B_w2,
):
    del B_x
    anyspec = pl.BlockSpec(memory_space=pl.ANY)
    out = pl.pallas_call(
        _kernel,
        in_specs=[anyspec] * 7,
        out_specs=anyspec,
        out_shape=jax.ShapeDtypeStruct((S, D), BF),
        scratch_shapes=[
            pltpu.VMEM((S, D), BF),
            pltpu.VMEM((D, 3 * D), BF),
            pltpu.VMEM((DH, DH, H), BF),
            pltpu.VMEM((D, D), BF),
            pltpu.VMEM((D, F), BF),
            pltpu.VMEM((D, F), BF),
            pltpu.VMEM((F, D), BF),
            pltpu.VMEM((S, D), BF),
            pltpu.VMEM((S // 128, 8, 128), F32),
            pltpu.VMEM((2 * D, D), BF),
            pltpu.VMEM((D, D), BF),
            pltpu.VMEM((32, D), F32),
            pltpu.VMEM((NG, GW + 8, 2 * GW), BF),
            pltpu.SemaphoreType.DMA((14,)),
            pltpu.SemaphoreType.DMA((NB, len(PIECES))),
        ],
        compiler_params=pltpu.CompilerParams(vmem_limit_bytes=100 * 1024 * 1024),
    )(A_x.reshape(S, D), A_wqkv, jnp.transpose(A_w_phi, (1, 2, 0)), A_wo, B_w1, B_w3, B_w2)
    return out.reshape(1, S, D)
```

```python
import jax
import jax.numpy as jnp
from jax import lax
import jax.experimental.pallas as pl
import jax.experimental.pallas.tpu as pltpu

S, D, H, DH, F = 2048, 640, 32, 20, 1536
NG = H // 2
GW = 2 * DH
NU = 6
NT3 = 11
TS = 512
NB = S // TS
HR = TS // 2
KP = (3, 2)
XP = (256, 128, 256, 768, 640)
DMA_ORDER = ('phi', 'k0', 'x0', 'k1', 'x1', 'v', 'x2', 'x3', 'x4', 'q', 'wo', 'w1', 'w3', 'w2')
PIECES = ((0, 0, D), (HR, 0, 256), (HR, 256, 256), (HR, 512, 128))
BF = jnp.bfloat16
F32 = jnp.float32
NT = (((1,), (1,)), ((), ()))
LOG2E = 1.4426950408889634


def _recip(x):
    r = pl.reciprocal(x, approx=True)
    return r * (2.0 - x * r)


def _swiglu(g, u):
    return g * u * _recip(1.0 + jnp.exp(jnp.minimum(-g, 80.0)))


def _zero(g):
    u = lax.bitcast_convert_type(g, jnp.uint32)
    u = lax.shift_right_logical(lax.shift_right_logical(u, jnp.uint32(16)), jnp.uint32(16))
    return lax.bitcast_convert_type(u, F32)


def _lanesum(x):
    s = x[:, 0:128]
    for t in range(1, x.shape[1] // 128):
        s = s + x[:, 128 * t:128 * (t + 1)]
    return s


def _layernorm(x, toks):
    n = x.shape[0] // len(toks)
    outs = []
    for j, tok in enumerate(toks):
        xj = x[n * j:n * (j + 1)]
        s = _lanesum(xj) + jnp.concatenate([_zero(tok)] * (n // 8), axis=0)
        xc = xj - jnp.sum(s, axis=-1, keepdims=True) * (1.0 / D)
        v = jnp.mean(xc * xc, axis=-1, keepdims=True)
        outs.append(xc * lax.rsqrt(v + 1e-5))
    return jnp.concatenate(outs, axis=0)


def _stats(x):
    s1 = jnp.sum(_lanesum(x).T.reshape(16, 8, 128), axis=0)
    s2 = jnp.sum(_lanesum(x * x).T.reshape(16, 8, 128), axis=0)
    for sh in (1, 2, 4):
        s1 = s1 + pltpu.roll(s1, sh, 0)
        s2 = s2 + pltpu.roll(s2, sh, 0)
    m = s1 * (1.0 / D)
    v = jnp.maximum(s2 * (1.0 / D) - m * m, 0.0)
    return m, lax.rsqrt(v + 1e-5)


def _allred(x, op):
    x = op(x, pltpu.roll(x, 2, 0))
    return op(x, pltpu.roll(x, 4, 0))


def _feature_map(p, sc, split):
    p3 = p.reshape(GW // 8, 8, 128) * sc[None]
    mx = _allred(jnp.max(p3, axis=0), jnp.maximum)
    mn = _allred(jnp.min(p3, axis=0), jnp.minimum)
    ep = jnp.exp2(p3 - mx[None])
    en = jnp.exp2(mn[None] - p3)
    rp = _recip(_allred(jnp.sum(ep, axis=0), jnp.add))
    rn = _recip(_allred(jnp.sum(en, axis=0), jnp.add))
    ep = ep * rp[None]
    en = en * rn[None]
    if split:
        even = (lax.broadcasted_iota(jnp.int32, (8, 128), 0) & 1) == 0
        en = jnp.stack([pltpu.roll(en[j], 1, 0) for j in range(GW // 8)])
        ep, en = jnp.where(even[None], ep, en), jnp.where(even[None], en, ep)
    return jnp.concatenate([ep, en], axis=0).reshape(2 * GW, 128)


def _phi_pair(phis):
    zero = jnp.zeros((8, phis[0].shape[1]), F32)
    return (jnp.concatenate([phis[0], phis[1][0:GW], zero], axis=0).astype(BF),
            jnp.concatenate([phis[1][GW:2 * GW], phis[2], zero], axis=0).astype(BF))


def _row(x, k):
    return jnp.broadcast_to(x[k:k + 1], x.shape)


def _kernel(x_hbm, wqkv_hbm, wphi_hbm, wo_hbm, w1_hbm, w3_hbm, w2_hbm, out_hbm,
            x_v, wqkv_v, wphi_v, wo_v, w1_v, w3_v, w2_v, out_v,
            rl_v, wkv_v, wq_v, a_v, kvt_v, kvl_v,
            sems, osems):
    def cp_w(c0, nc, s):
        return pltpu.make_async_copy(wqkv_hbm.at[:, pl.ds(c0, nc)], wqkv_v.at[:, pl.ds(c0, nc)], sems.at[s])

    cps = {'phi': pltpu.make_async_copy(wphi_hbm, wphi_v, sems.at[0])}
    for i, n in enumerate(KP):
        cps['k%d' % i] = cp_w(D + 128 * sum(KP[:i]), 128 * n, 1 + i)
    for i, n in enumerate(XP):
        rows = pl.ds(sum(XP[:i]), n)
        cps['x%d' % i] = pltpu.make_async_copy(x_hbm.at[rows], x_v.at[rows], sems.at[3 + i])
    cps['v'] = cp_w(2 * D, D, 8)
    cps['q'] = cp_w(0, D, 9)
    cps['wo'] = pltpu.make_async_copy(wo_hbm, wo_v, sems.at[10])
    cps['w1'] = pltpu.make_async_copy(w1_hbm, w1_v, sems.at[11])
    cps['w3'] = pltpu.make_async_copy(w3_hbm, w3_v, sems.at[12])
    cps['w2'] = pltpu.make_async_copy(w2_hbm, w2_v, sems.at[13])
    for name in DMA_ORDER:
        cps[name].start()

    def wait(*names):
        for name in names:
            cps[name].wait()

    a_v[...] = jnp.zeros(a_v.shape, F32)
    j = lax.broadcasted_iota(jnp.int32, (D, D), 0)
    c = lax.broadcasted_iota(jnp.int32, (D, D), 1)
    perm = jnp.where(c == (j & 31) * DH + (j >> 5), 1.0, 0.0).astype(BF)
    r = lax.broadcasted_iota(jnp.int32, (GW, 32), 0)
    c = lax.broadcasted_iota(jnp.int32, (GW, 32), 1)
    esel = jnp.where(c == (r >> 1), 1.0, 0.0).astype(BF)
    wait('phi')
    for d in range(DH):
        a_v[0:DH, 32 * d:32 * (d + 1)] = wphi_v[d].astype(F32)
    a2 = jnp.dot(a_v[...].astype(BF), perm, preferred_element_type=F32).astype(BF)
    t40 = jnp.dot(esel, a2, preferred_element_type=F32)
    r = lax.broadcasted_iota(jnp.int32, (GW, 128), 0)
    c = lax.broadcasted_iota(jnp.int32, (GW, 128), 1)
    pts = []
    for t in range(5):
        blocks = []
        for jj in range(4):
            lo = ((r & 1) + 2 * (3 * t + jj)) * DH - 128 * t
            blocks.append(jnp.where((c >= lo) & (c < lo + DH), t40[:, 128 * t:128 * (t + 1)], 0.0))
        pts.append(jnp.concatenate(blocks, axis=0).astype(BF))

    def fold(dst, col0, t0, t1, state):
        row, done, carry = state
        for t in range(t0, t1):
            rt = lax.dot_general(pts[t], wqkv_v[:, col0 + 128 * t:col0 + 128 * (t + 1)], NT,
                                 preferred_element_type=F32)
            done = done + [rt[0:GW] if carry is None else rt[0:GW] + carry, rt[GW:160 if t == 4 else 120]]
            carry = rt[120:160]
        w = jnp.concatenate(done, axis=0)
        n = w.shape[0] // 80 * 80
        wn = w[0:n]
        dst[row:row + n, :] = (wn - jnp.sum(_lanesum(wn), axis=-1, keepdims=True) * (1.0 / D)).astype(BF)
        return row + n, [w[n:]] if n < w.shape[0] else [], carry

    def proj(w_v, g0, ng, x):
        return lax.dot_general(w_v[GW * g0:GW * (g0 + ng), :], x, NT, preferred_element_type=F32)

    acc = [None] * NT3
    pks, pvs, phis, rs, rls, exs = {}, {}, {}, {}, {}, {}
    low8 = lax.broadcasted_iota(jnp.int32, (8, 128), 0) < 4
    even8 = (lax.broadcasted_iota(jnp.int32, (8, 128), 0) & 1) == 0

    def stats(t0, t1):
        for t in range(t0, t1):
            m, rs[t] = _stats(x_v[128 * t:128 * (t + 1), :].astype(F32))
            exs[t] = jnp.where(even8, 1.0, m * rs[t])
            rls[t] = rs[t] * LOG2E
            rl_v[t] = rls[t]

    def kv_proj(dst, base, t0, t1, g0, g1):
        p = proj(wkv_v, base + g0, g1 - g0, x_v[128 * t0:128 * t1, :])
        for g in range(g0, g1):
            for t in range(t0, t1):
                dst[t, g] = p[GW * (g - g0):GW * (g - g0 + 1), 128 * (t - t0):128 * (t - t0 + 1)]

    def kproj(t0, t1, g0=0, g1=NG):
        kv_proj(pks, 0, t0, t1, g0, g1)

    def vproj(t0, t1, g0=0, g1=NG):
        kv_proj(pvs, NG, t0, t1, g0, g1)

    def feat(t0, t1, g0=0, g1=NG):
        for t in range(t0, t1):
            for g in range(g0, g1):
                phis[t, g] = _feature_map(pks[t, g], rls[t], g % 3 == 1)

    def accum(t0, t1, u0=0, u1=NU):
        ts = range(t0, t1)
        for u in range(u0, u1):
            gs = range(3 * u, min(3 * u + 3, NG))
            phi = [jnp.concatenate([phis[t, g] for t in ts], axis=1) for g in gs]
            vts = []
            for t in ts:
                v = jnp.concatenate([pvs[t, g] for g in gs], axis=0)
                v = (v.reshape(v.shape[0] // 8, 8, 128) * rs[t][None]).reshape(v.shape)
                if u < NU - 1:
                    vts.append(jnp.concatenate([v[0:56], jnp.where(low8, v[56:64], exs[t]),
                                                jnp.where(low8, exs[t], v[56:64]), v[64:120]], axis=0))
                else:
                    vts.append(jnp.concatenate([v, exs[t]], axis=0))
            vt = jnp.concatenate(vts, axis=1)
            if u < NU - 1:
                pairs = zip((vt[0:64], vt[64:128]), _phi_pair(phi))
            else:
                pairs = [(vt, phi[0].astype(BF))]
            for k, (lhs, rhs) in enumerate(pairs):
                kv = lax.dot_general(lhs.astype(BF), rhs, NT, preferred_element_type=F32)
                acc[2 * u + k] = kv if acc[2 * u + k] is None else kv + acc[2 * u + k]

    wait('k0')
    fk = fold(wkv_v, D, 0, KP[0], (0, [], None))
    wait('x0')
    stats(0, 2)
    kproj(0, 2, 0, 4)
    feat(0, 2, 0, 4)
    kproj(0, 2, 4, 8)
    wait('k1', 'x1')
    fold(wkv_v, D, KP[0], 5, fk)
    stats(2, 3)
    kproj(2, 3, 0, 8)
    feat(0, 2, 4, 8)
    kproj(0, 3, 8, 16)
    wait('v', 'x2')
    wkv_v[D:2 * D, :] = wqkv_v[:, 2 * D:3 * D].T
    stats(3, 5)
    for g in range(0, NG, 4):
        kproj(3, 5, g, g + 4)
    vproj(0, 4, 0, 4)
    feat(2, 3, 0, 8)
    feat(0, 3, 8, 9)
    vproj(0, 4, 4, 8)
    feat(0, 3, 9, 13)
    vproj(0, 4, 8, 12)
    feat(0, 3, 13, 16)
    feat(3, 4, 0, 4)
    vproj(0, 4, 12, 16)
    wait('x3', 'x4', 'q')
    wv_sum = jnp.sum(_lanesum(wkv_v[D:2 * D, :].astype(F32)), axis=-1, keepdims=True)
    stats(5, 8)
    for g in range(0, NG, 4):
        kproj(5, 8, g, g + 4)
    feat(3, 4, 4, 16)
    feat(4, 8)
    for t in (4, 8, 12):
        if t > 4:
            kproj(t, t + 4)
            feat(t, t + 4)
        if t < 12:
            stats(t + 4, t + 8)
        for q, (u0, u1) in enumerate(((0, 1), (1, 3), (3, 4), (4, 6))):
            vproj(t, t + 4, 4 * q, 4 * q + 4)
            accum(t - 4, t, u0, u1)
    accum(12, 16, 0, 3)
    fold(wq_v, 0, 0, 5, (0, [], None))
    accum(12, 16, 3, 6)

    r = lax.broadcasted_iota(jnp.int32, (64, 128), 0)
    c = lax.broadcasted_iota(jnp.int32, (64, 128), 1)

    def rhead(r):
        return jnp.where(r >= 2 * DH, 2, jnp.where(r >= DH, 1, 0))

    pad = c >= 3 * GW
    msks = [jnp.where(r < 60, rhead(r), r - 60) == jnp.where(pad, -1, jnp.where(c < 2 * GW, c & 1, 2)),
            jnp.where(r < 4, r, rhead(r - 4)) == jnp.where(pad, -1, jnp.where(c < GW, 0, 1 + (c & 1)))]
    isz = [r >= 60, r < 4]
    for j in range(NT3 - 1):
        k = j % 2
        row = 60 * j - 4 * k
        zt = acc[j][60 * (1 - k):60 * (1 - k) + 1]
        mt = acc[j][60 * (1 - k) + 1:60 * (1 - k) + 2]
        kv = jnp.where(isz[k], zt, acc[j] - wv_sum[row:row + 64] * mt)
        kvt_v[j] = jnp.where(msks[k], kv, 0.0).astype(BF)
    r = lax.broadcasted_iota(jnp.int32, (GW + 8, 2 * GW), 0)
    c = lax.broadcasted_iota(jnp.int32, (GW + 8, 2 * GW), 1)
    last = acc[NT3 - 1]
    kv = jnp.concatenate([last[0:GW] - wv_sum[D - GW:D] * last[GW + 1:GW + 2],
                          jnp.broadcast_to(last[GW:GW + 1], (8, 2 * GW))], axis=0)
    hh = jnp.where(r < GW, jnp.where(r >= DH, 1, 0), jnp.where(r >= GW + 4, 1, 0))
    kvl_v[...] = jnp.where(hh == (c & 1), kv, 0.0).astype(BF)
    wait('wo', 'w1', 'w3', 'w2')

    def cp_out(i, p):
        r0, c0, nc = PIECES[p]
        rows = pl.ds(pl.multiple_of(i * TS + r0, HR), HR)
        return pltpu.make_async_copy(out_v.at[rows, pl.ds(c0, nc)], out_hbm.at[rows, pl.ds(c0, nc)], osems.at[i, p])

    def phase2(i, carry):
        row0 = pl.multiple_of(i * TS, TS)
        scs = [rl_v[(TS // 128) * i + t] for t in range(TS // 128)]
        low = lax.broadcasted_iota(jnp.int32, (8, TS), 0) < 4
        pq = proj(wq_v, 0, NG, x_v[pl.ds(row0, TS), :])
        ots = []
        for u in range(NU):
            phi = [jnp.concatenate([_feature_map(pq[GW * g:GW * (g + 1), 128 * t:128 * (t + 1)], scs[t], g % 3 == 1)
                                    for t in range(TS // 128)], axis=1) for g in range(3 * u, min(3 * u + 3, NG))]
            if u < NU - 1:
                phia, phib = _phi_pair(phi)
                na = jnp.dot(kvt_v[2 * u], phia, preferred_element_type=F32)
                nb = jnp.dot(kvt_v[2 * u + 1], phib, preferred_element_type=F32)
                rd = _recip(jnp.where(low, nb[0:8], na[56:64]) + 1e-6)
                nd = jnp.concatenate([na[0:56], jnp.where(low, na[56:64], nb[0:8]), nb[8:64]], axis=0)
                rh = [_row(rd, k) for k in (4, 5, 6, 0, 1, 2)]
            else:
                nd = jnp.dot(kvl_v[...], phi[0].astype(BF), preferred_element_type=F32)
                rd = _recip(nd[GW:GW + 8] + 1e-6)
                rr = pltpu.roll(rd, 4, 0)
                rh = [jnp.where(low, rd, rr), jnp.where(low, rr, rd)]
            for j in range(len(rh) // 2):
                ra, rb = rh[2 * j], rh[2 * j + 1]
                for k, sc in enumerate((ra, ra, jnp.where(low, ra, rb), rb, rb)):
                    ots.append(nd[GW * j + 8 * k:GW * j + 8 * (k + 1)] * sc)
        ot = jnp.concatenate(ots, axis=0)
        hs, atts, acts = [], [], []
        for p in range(2):
            o = ot[:, HR * p:HR * (p + 1)].T.astype(BF)
            atts.append(jnp.dot(o, wo_v[...], preferred_element_type=F32))
            hs.append(x_v[pl.ds(pl.multiple_of(row0 + HR * p, HR), HR), :].astype(F32) + atts[-1])
        toks = [atts[1][HR - 8:HR, 128 * t:128 * (t + 1)] for t in range(4)]
        for p in range(2):
            hn = _layernorm(hs[p], toks).astype(BF)
            gate = jnp.dot(hn, w1_v[...], preferred_element_type=F32)
            up = jnp.dot(hn, w3_v[...], preferred_element_type=F32)
            acts.append(_swiglu(gate, up))
            toks = [gate[HR - 8:HR, 128 * t:128 * (t + 1)] for t in range(8)]
        actb = {}
        for p, (r0, c0, nc) in enumerate(PIECES):
            hp = r0 // HR
            if hp not in actb:
                actb[hp] = acts[hp].astype(BF)
            y = hs[hp][:, c0:c0 + nc] + jnp.dot(actb[hp], w2_v[:, c0:c0 + nc], preferred_element_type=F32)
            out_v[pl.ds(pl.multiple_of(row0 + r0, HR), HR), c0:c0 + nc] = y.astype(BF)
            cp_out(i, p).start()
        return carry

    lax.fori_loop(0, NB, phase2, 0)
    for i in range(NB):
        for p in range(len(PIECES)):
            cp_out(i, p).wait()


@jax.jit
def pallas_sequential_preLN__linear_kernel_hedgehog__glu_gated_swiglu__prompt_kernel(
    A_x, A_wqkv, A_w_phi, A_wo, B_x, B_w1, B_w3, B_w2,
):
    del B_x
    anyspec = pl.BlockSpec(memory_space=pl.ANY)
    out = pl.pallas_call(
        _kernel,
        in_specs=[anyspec] * 7,
        out_specs=anyspec,
        out_shape=jax.ShapeDtypeStruct((S, D), BF),
        scratch_shapes=[
            pltpu.VMEM((S, D), BF),
            pltpu.VMEM((D, 3 * D), BF),
            pltpu.VMEM((DH, DH, H), BF),
            pltpu.VMEM((D, D), BF),
            pltpu.VMEM((D, F), BF),
            pltpu.VMEM((D, F), BF),
            pltpu.VMEM((F, D), BF),
            pltpu.VMEM((S, D), BF),
            pltpu.VMEM((S // 128, 8, 128), F32),
            pltpu.VMEM((2 * D, D), BF),
            pltpu.VMEM((D, D), BF),
            pltpu.VMEM((32, D), F32),
            pltpu.VMEM((NT3 - 1, 64, 128), BF),
            pltpu.VMEM((GW + 8, 2 * GW), BF),
            pltpu.SemaphoreType.DMA((14,)),
            pltpu.SemaphoreType.DMA((NB, len(PIECES))),
        ],
        compiler_params=pltpu.CompilerParams(vmem_limit_bytes=100 * 1024 * 1024),
    )(A_x.reshape(S, D), A_wqkv, jnp.transpose(A_w_phi, (1, 2, 0)), A_wo, B_w1, B_w3, B_w2)
    return out.reshape(1, S, D)
```

```python
import jax
import jax.numpy as jnp
from jax import lax
import jax.experimental.pallas as pl
import jax.experimental.pallas.tpu as pltpu

S, D, H, DH, F = 2048, 640, 32, 20, 1536
NG = H // 2
GW = 2 * DH
NU = 6
NT3 = 11
TS = 512
NB = S // TS
HR = TS // 2
KP = (3, 2)
XP = (256, 128, 256, 768, 640)
DMA_ORDER = ('phi', 'k0', 'x0', 'k1', 'x1', 'v', 'x2', 'x3', 'x4', 'q', 'wo', 'w1', 'w3', 'w2')
PIECES = ((0, 0, D, 1), (HR, 0, 256, 1), (HR, 256, 256, 2), (HR, 512, 128, 4))
PLAN = (
    ('s', 5, 8), ('k', 5, 8, 0, 4), ('f', 4, 8, 0, 4), ('k', 5, 8, 4, 8), ('f', 3, 4, 4, 8), ('k', 5, 8, 8, 12),
    ('f', 3, 4, 8, 12), ('f', 4, 8, 4, 8), ('f', 4, 8, 8, 12), ('k', 5, 8, 12, 16), ('v', 5, 8, 0, 4), ('a', 0,
    4, 0, 1), ('f', 4, 8, 12, 16), ('f', 3, 4, 12, 16), ('s', 8, 9), ('v', 5, 8, 4, 8), ('s', 9, 10), ('v', 5,
    8, 8, 12), ('s', 10, 11), ('s', 11, 12), ('a', 0, 4, 1, 2), ('a', 0, 4, 2, 3), ('a', 0, 4, 3, 4), ('v', 5,
    8, 12, 16), ('a', 0, 4, 4, 5), ('a', 0, 4, 5, 6), ('k', 8, 12, 4, 8), ('k', 8, 12, 0, 4), ('k', 8, 12, 8,
    12), ('k', 8, 12, 12, 16), ('v', 8, 12, 0, 4), ('f', 8, 12), ('s', 12, 13), ('x', 9, 10), ('a', 4, 8, 0, 1),
    ('a', 4, 8, 1, 2), ('a', 4, 8, 4, 5), ('a', 4, 8, 2, 3), ('s', 13, 14), ('a', 4, 8, 3, 4), ('v', 8, 12, 4,
    8), ('x', 5, 6), ('x', 6, 7), ('s', 14, 15), ('a', 4, 8, 5, 6), ('v', 8, 12, 8, 12), ('x', 7, 8), ('k', 12,
    16, 8, 16), ('k', 12, 16, 0, 8), ('s', 15, 16), ('x', 8, 9), ('f', 12, 16), ('v', 12, 16, 0, 4), ('v', 8,
    12, 12, 16), ('a', 8, 12, 0, 1), ('x', 14, 15), ('a', 8, 12, 1, 2), ('x', 10, 11), ('a', 8, 12, 5, 6), ('v',
    12, 16, 4, 8), ('x', 11, 12), ('x', 15, 16), ('v', 12, 16, 8, 12), ('a', 8, 12, 2, 3), ('a', 8, 12, 3, 4),
    ('v', 12, 16, 12, 16), ('x', 12, 13), ('x', 13, 14), ('a', 8, 12, 4, 5), ('a', 12, 16, 0, 1), ('a', 12, 16,
    1, 2), ('q',), ('a', 12, 16, 3, 4), ('a', 12, 16, 4, 5), ('a', 12, 16, 5, 6), ('a', 12, 16, 2, 3))
PACE0 = tuple((t, r) for t in range(4) for r in (6, 14, 22, 30))
PACE1 = ((1, 23), (1, 31), (2, 31), (3, 23), (4, 31), (5, 31), (6, 31), (7, 23))
BF = jnp.bfloat16
F32 = jnp.float32
NT = (((1,), (1,)), ((), ()))
LOG2E = 1.4426950408889634


def _recip(x):
    r = pl.reciprocal(x, approx=True)
    return r * (2.0 - x * r)


def _swiglu(g, u):
    return g * u * _recip(1.0 + jnp.exp(jnp.minimum(-g, 80.0)))


def _zero(g):
    u = lax.bitcast_convert_type(g, jnp.uint32)
    u = lax.shift_right_logical(lax.shift_right_logical(u, jnp.uint32(16)), jnp.uint32(16))
    return lax.bitcast_convert_type(u, F32)


def _lanesum(x):
    s = x[:, 0:128]
    for t in range(1, x.shape[1] // 128):
        s = s + x[:, 128 * t:128 * (t + 1)]
    return s


def _layernorm(x, toks):
    n = x.shape[0] // len(toks)
    outs = []
    for j, tok in enumerate(toks):
        xj = x[n * j:n * (j + 1)]
        s = _lanesum(xj) + jnp.concatenate([_zero(tok)] * (n // 8), axis=0)
        xc = xj - jnp.sum(s, axis=-1, keepdims=True) * (1.0 / D)
        v = jnp.mean(xc * xc, axis=-1, keepdims=True)
        outs.append(xc * lax.rsqrt(v + 1e-5))
    return jnp.concatenate(outs, axis=0)


def _stats(x):
    s1 = jnp.sum(_lanesum(x).T.reshape(16, 8, 128), axis=0)
    s2 = jnp.sum(_lanesum(x * x).T.reshape(16, 8, 128), axis=0)
    for sh in (1, 2, 4):
        s1 = s1 + pltpu.roll(s1, sh, 0)
        s2 = s2 + pltpu.roll(s2, sh, 0)
    m = s1 * (1.0 / D)
    v = jnp.maximum(s2 * (1.0 / D) - m * m, 0.0)
    return m, lax.rsqrt(v + 1e-5)


def _allred(x, op):
    x = op(x, pltpu.roll(x, 2, 0))
    return op(x, pltpu.roll(x, 4, 0))


def _feature_map(p, sc, split):
    p3 = p.reshape(GW // 8, 8, 128) * sc[None]
    mx = _allred(jnp.max(p3, axis=0), jnp.maximum)
    mn = _allred(jnp.min(p3, axis=0), jnp.minimum)
    ep = jnp.exp2(p3 - mx[None])
    en = jnp.exp2(mn[None] - p3)
    rp = _recip(_allred(jnp.sum(ep, axis=0), jnp.add))
    rn = _recip(_allred(jnp.sum(en, axis=0), jnp.add))
    ep = ep * rp[None]
    en = en * rn[None]
    if split:
        even = (lax.broadcasted_iota(jnp.int32, (8, 128), 0) & 1) == 0
        en = jnp.stack([pltpu.roll(en[j], 1, 0) for j in range(GW // 8)])
        ep, en = jnp.where(even[None], ep, en), jnp.where(even[None], en, ep)
    return jnp.concatenate([ep, en], axis=0).reshape(2 * GW, 128)


def _phi_pair(phis):
    zero = jnp.zeros((8, phis[0].shape[1]), F32)
    return (jnp.concatenate([phis[0], phis[1][0:GW], zero], axis=0).astype(BF),
            jnp.concatenate([phis[1][GW:2 * GW], phis[2], zero], axis=0).astype(BF))


def _row(x, k):
    return jnp.broadcast_to(x[k:k + 1], x.shape)


def _kernel(x_hbm, wqkv_hbm, wphi_hbm, wo_hbm, w1_hbm, w3_hbm, w2_hbm, out_hbm,
            x_v, wqkv_v, wphi_v, wo_v, w1_v, w3_v, w2_v, out_v,
            rl_v, xt_v, wkv_v, wq_v, a_v, kvt_v, kvl_v,
            sems, osems):
    def cp_w(c0, nc, s):
        return pltpu.make_async_copy(wqkv_hbm.at[:, pl.ds(c0, nc)], wqkv_v.at[:, pl.ds(c0, nc)], sems.at[s])

    cps = {'phi': pltpu.make_async_copy(wphi_hbm, wphi_v, sems.at[0])}
    for i, n in enumerate(KP):
        cps['k%d' % i] = cp_w(D + 128 * sum(KP[:i]), 128 * n, 1 + i)
    for i, n in enumerate(XP):
        rows = pl.ds(sum(XP[:i]), n)
        cps['x%d' % i] = pltpu.make_async_copy(x_hbm.at[rows], x_v.at[rows], sems.at[3 + i])
    cps['v'] = cp_w(2 * D, D, 8)
    cps['q'] = cp_w(0, D, 9)
    cps['wo'] = pltpu.make_async_copy(wo_hbm, wo_v, sems.at[10])
    cps['w1'] = pltpu.make_async_copy(w1_hbm, w1_v, sems.at[11])
    cps['w3'] = pltpu.make_async_copy(w3_hbm, w3_v, sems.at[12])
    cps['w2'] = pltpu.make_async_copy(w2_hbm, w2_v, sems.at[13])
    for name in DMA_ORDER:
        cps[name].start()

    def wait(*names):
        for name in names:
            cps[name].wait()

    a_v[...] = jnp.zeros(a_v.shape, F32)
    j = lax.broadcasted_iota(jnp.int32, (D, D), 0)
    c = lax.broadcasted_iota(jnp.int32, (D, D), 1)
    perm = jnp.where(c == (j & 31) * DH + (j >> 5), 1.0, 0.0).astype(BF)
    r = lax.broadcasted_iota(jnp.int32, (GW, 32), 0)
    c = lax.broadcasted_iota(jnp.int32, (GW, 32), 1)
    esel = jnp.where(c == (r >> 1), 1.0, 0.0).astype(BF)
    wait('phi')
    for d in range(DH):
        a_v[0:DH, 32 * d:32 * (d + 1)] = wphi_v[d].astype(F32)
    a2 = jnp.dot(a_v[...].astype(BF), perm, preferred_element_type=F32).astype(BF)
    t40 = jnp.dot(esel, a2, preferred_element_type=F32)
    r = lax.broadcasted_iota(jnp.int32, (GW, 128), 0)
    c = lax.broadcasted_iota(jnp.int32, (GW, 128), 1)
    pts = []
    for t in range(5):
        blocks = []
        for jj in range(4):
            lo = ((r & 1) + 2 * (3 * t + jj)) * DH - 128 * t
            blocks.append(jnp.where((c >= lo) & (c < lo + DH), t40[:, 128 * t:128 * (t + 1)], 0.0))
        pts.append(jnp.concatenate(blocks, axis=0).astype(BF))

    def fold(dst, col0, t0, t1, state):
        row, done, carry = state
        for t in range(t0, t1):
            rt = lax.dot_general(pts[t], wqkv_v[:, col0 + 128 * t:col0 + 128 * (t + 1)], NT,
                                 preferred_element_type=F32)
            done = done + [rt[0:GW] if carry is None else rt[0:GW] + carry, rt[GW:160 if t == 4 else 120]]
            carry = rt[120:160]
        w = jnp.concatenate(done, axis=0)
        n = w.shape[0] // 80 * 80
        wn = w[0:n]
        dst[row:row + n, :] = (wn - jnp.sum(_lanesum(wn), axis=-1, keepdims=True) * (1.0 / D)).astype(BF)
        return row + n, [w[n:]] if n < w.shape[0] else [], carry

    def proj(w_v, g0, ng, x):
        return lax.dot_general(w_v[GW * g0:GW * (g0 + ng), :], x, NT, preferred_element_type=F32)

    acc = [None] * NT3
    pks, pvs, phis, rs, rls, exs = {}, {}, {}, {}, {}, {}
    low8 = lax.broadcasted_iota(jnp.int32, (8, 128), 0) < 4
    even8 = (lax.broadcasted_iota(jnp.int32, (8, 128), 0) & 1) == 0

    def stats(t0, t1):
        for t in range(t0, t1):
            m, rs[t] = _stats(x_v[128 * t:128 * (t + 1), :].astype(F32))
            exs[t] = jnp.where(even8, 1.0, m * rs[t])
            rls[t] = rs[t] * LOG2E
            rl_v[t] = rls[t]

    def xtr(t0, t1):
        for t in range(t0, t1):
            xt_v[t // 4, :, 128 * (t % 4):128 * (t % 4 + 1)] = x_v[128 * t:128 * (t + 1), 0:128].T

    def kv_proj(dst, base, t0, t1, g0, g1):
        p = proj(wkv_v, base + g0, g1 - g0, x_v[128 * t0:128 * t1, :])
        for g in range(g0, g1):
            for t in range(t0, t1):
                dst[t, g] = p[GW * (g - g0):GW * (g - g0 + 1), 128 * (t - t0):128 * (t - t0 + 1)]

    def kproj(t0, t1, g0=0, g1=NG):
        kv_proj(pks, 0, t0, t1, g0, g1)

    def vproj(t0, t1, g0=0, g1=NG):
        kv_proj(pvs, NG, t0, t1, g0, g1)

    def vhead(pv):
        pv = jnp.dot(wkv_v[D + 480:2 * D, 0:128], xt_v[0], preferred_element_type=F32) + pv
        for g in range(12, NG):
            for t in range(4):
                pvs[t, g] = pv[GW * (g - 12):GW * (g - 11), 128 * t:128 * (t + 1)]

    def feat(t0, t1, g0=0, g1=NG):
        for t in range(t0, t1):
            for g in range(g0, g1):
                phis[t, g] = _feature_map(pks[t, g], rls[t], g % 3 == 1)

    def accum(t0, t1, u0=0, u1=NU):
        ts = range(t0, t1)
        for u in range(u0, u1):
            gs = range(3 * u, min(3 * u + 3, NG))
            phi = [jnp.concatenate([phis[t, g] for t in ts], axis=1) for g in gs]
            vts = []
            for t in ts:
                v = jnp.concatenate([pvs[t, g] for g in gs], axis=0)
                v = (v.reshape(v.shape[0] // 8, 8, 128) * rs[t][None]).reshape(v.shape)
                if u < NU - 1:
                    vts.append(jnp.concatenate([v[0:56], jnp.where(low8, v[56:64], exs[t]),
                                                jnp.where(low8, exs[t], v[56:64]), v[64:120]], axis=0))
                else:
                    vts.append(jnp.concatenate([v, exs[t]], axis=0))
            vt = jnp.concatenate(vts, axis=1)
            if u < NU - 1:
                pairs = zip((vt[0:64], vt[64:128]), _phi_pair(phi))
            else:
                pairs = [(vt, phi[0].astype(BF))]
            for k, (lhs, rhs) in enumerate(pairs):
                kv = lax.dot_general(lhs.astype(BF), rhs, NT, preferred_element_type=F32)
                acc[2 * u + k] = kv if acc[2 * u + k] is None else kv + acc[2 * u + k]

    wait('k0')
    fk = fold(wkv_v, D, 0, KP[0], (0, [], None))
    wait('x0')
    stats(0, 2)
    kproj(0, 2, 0, 4)
    feat(0, 2, 0, 4)
    kproj(0, 2, 4, 8)
    wait('k1', 'x1')
    fold(wkv_v, D, KP[0], 5, fk)
    stats(2, 3)
    kproj(2, 3, 0, 8)
    feat(0, 2, 4, 8)
    kproj(0, 3, 8, 16)
    wait('v', 'x2')
    for c0 in range(0, D, 128):
        wkv_v[D + c0:D + c0 + 128, :] = wqkv_v[:, 2 * D + c0:2 * D + c0 + 128].T
    stats(3, 5)
    for g in range(0, NG, 4):
        kproj(3, 5, g, g + 4)
    vproj(0, 5, 0, 4)
    feat(2, 3, 0, 8)
    feat(0, 3, 8, 9)
    vproj(0, 5, 4, 8)
    feat(0, 3, 9, 13)
    vproj(0, 5, 8, 12)
    feat(0, 3, 13, 16)
    feat(3, 4, 0, 4)
    vproj(4, 5, 12, 16)
    pv = lax.dot_general(wkv_v[D + 480:2 * D, 128:D], x_v[0:TS, 128:D], NT, preferred_element_type=F32)
    xtr(0, 5)
    wv_sum = jnp.sum(_lanesum(wkv_v[D:2 * D, :].astype(F32)), axis=-1, keepdims=True)
    wait('x3', 'x4', 'q')
    vhead(pv)
    steps = {'s': stats, 'k': kproj, 'v': vproj, 'f': feat, 'a': accum, 'x': xtr,
             'q': lambda: fold(wq_v, 0, 0, 5, (0, [], None))}
    for kind, *args in PLAN:
        steps[kind](*args)

    r = lax.broadcasted_iota(jnp.int32, (64, 128), 0)
    c = lax.broadcasted_iota(jnp.int32, (64, 128), 1)

    def rhead(r):
        return jnp.where(r >= 2 * DH, 2, jnp.where(r >= DH, 1, 0))

    pad = c >= 3 * GW
    msks = [jnp.where(r < 60, rhead(r), r - 60) == jnp.where(pad, -1, jnp.where(c < 2 * GW, c & 1, 2)),
            jnp.where(r < 4, r, rhead(r - 4)) == jnp.where(pad, -1, jnp.where(c < GW, 0, 1 + (c & 1)))]
    isz = [r >= 60, r < 4]
    for j in range(NT3 - 1):
        k = j % 2
        row = 60 * j - 4 * k
        zt = acc[j][60 * (1 - k):60 * (1 - k) + 1]
        mt = acc[j][60 * (1 - k) + 1:60 * (1 - k) + 2]
        kv = jnp.where(isz[k], zt, acc[j] - wv_sum[row:row + 64] * mt)
        kvt_v[j] = jnp.where(msks[k], kv, 0.0).astype(BF)
    r = lax.broadcasted_iota(jnp.int32, (GW + 8, 2 * GW), 0)
    c = lax.broadcasted_iota(jnp.int32, (GW + 8, 2 * GW), 1)
    last = acc[NT3 - 1]
    kv = jnp.concatenate([last[0:GW] - wv_sum[D - GW:D] * last[GW + 1:GW + 2],
                          jnp.broadcast_to(last[GW:GW + 1], (8, 2 * GW))], axis=0)
    hh = jnp.where(r < GW, jnp.where(r >= DH, 1, 0), jnp.where(r >= GW + 4, 1, 0))
    kvl_v[...] = jnp.where(hh == (c & 1), kv, 0.0).astype(BF)
    wait('wo', 'w1', 'w3', 'w2')

    def cp_out(i, p, q):
        r0, c0, nc, ns = PIECES[p]
        rows = pl.ds(pl.multiple_of(i * TS + r0 + HR // ns * q, HR // ns), HR // ns)
        sem = osems.at[i, sum(pc[3] for pc in PIECES[:p]) + q]
        return pltpu.make_async_copy(out_v.at[rows, pl.ds(c0, nc)], out_hbm.at[rows, pl.ds(c0, nc)], sem)

    def phase2(i, carry):
        row0 = pl.multiple_of(i * TS, TS)
        scs = [rl_v[(TS // 128) * i + t] for t in range(TS // 128)]
        low = lax.broadcasted_iota(jnp.int32, (8, TS), 0) < 4
        pq = jnp.dot(wq_v[:, 0:128], xt_v[i], preferred_element_type=F32)
        pq = lax.dot_general(wq_v[:, 128:D], x_v[pl.ds(row0, TS), 128:D], NT, preferred_element_type=F32) + pq
        ots = []
        for u in range(NU):
            phi = [jnp.concatenate([_feature_map(pq[GW * g:GW * (g + 1), 128 * t:128 * (t + 1)], scs[t], g % 3 == 1)
                                    for t in range(TS // 128)], axis=1) for g in range(3 * u, min(3 * u + 3, NG))]
            if u < NU - 1:
                phia, phib = _phi_pair(phi)
                na = jnp.dot(kvt_v[2 * u], phia, preferred_element_type=F32)
                nb = jnp.dot(kvt_v[2 * u + 1], phib, preferred_element_type=F32)
                rd = _recip(jnp.where(low, nb[0:8], na[56:64]) + 1e-6)
                nd = jnp.concatenate([na[0:56], jnp.where(low, na[56:64], nb[0:8]), nb[8:64]], axis=0)
                rh = [_row(rd, k) for k in (4, 5, 6, 0, 1, 2)]
            else:
                nd = jnp.dot(kvl_v[...], phi[0].astype(BF), preferred_element_type=F32)
                rd = _recip(nd[GW:GW + 8] + 1e-6)
                rr = pltpu.roll(rd, 4, 0)
                rh = [jnp.where(low, rd, rr), jnp.where(low, rr, rd)]
            for j in range(len(rh) // 2):
                ra, rb = rh[2 * j], rh[2 * j + 1]
                for k, sc in enumerate((ra, ra, jnp.where(low, ra, rb), rb, rb)):
                    ots.append(nd[GW * j + 8 * k:GW * j + 8 * (k + 1)] * sc)
        ot = jnp.concatenate(ots, axis=0)
        hs, atts, acts = [], [], []
        for p in range(2):
            o = ot[:, HR * p:HR * (p + 1)].T.astype(BF)
            atts.append(jnp.dot(o, wo_v[...], preferred_element_type=F32))
            hs.append(x_v[pl.ds(pl.multiple_of(row0 + HR * p, HR), HR), :].astype(F32) + atts[-1])
        toks = [atts[1][8 * r:8 * r + 8, 128 * t:128 * (t + 1)] for t, r in PACE0]
        for p in range(2):
            hn = _layernorm(hs[p], toks).astype(BF)
            gate = jnp.dot(hn, w1_v[...], preferred_element_type=F32)
            up = jnp.dot(hn, w3_v[...], preferred_element_type=F32)
            acts.append(_swiglu(gate, up))
            toks = [gate[8 * r:8 * r + 8, 128 * t:128 * (t + 1)] for t, r in PACE1]
        actb = {}
        for p, (r0, c0, nc, ns) in enumerate(PIECES):
            hp = r0 // HR
            if hp not in actb:
                actb[hp] = acts[hp].astype(BF)
            y = hs[hp][:, c0:c0 + nc] + jnp.dot(actb[hp], w2_v[:, c0:c0 + nc], preferred_element_type=F32)
            n = HR // ns
            for q in range(ns):
                out_v[pl.ds(pl.multiple_of(row0 + r0 + n * q, n), n), c0:c0 + nc] = y[n * q:n * (q + 1)].astype(BF)
                cp_out(i, p, q).start()
        return carry

    lax.fori_loop(0, NB, phase2, 0)
    for i in range(NB):
        for p, pc in enumerate(PIECES):
            for q in range(pc[3]):
                cp_out(i, p, q).wait()


@jax.jit
def pallas_sequential_preLN__linear_kernel_hedgehog__glu_gated_swiglu__prompt_kernel(
    A_x, A_wqkv, A_w_phi, A_wo, B_x, B_w1, B_w3, B_w2,
):
    del B_x
    anyspec = pl.BlockSpec(memory_space=pl.ANY)
    out = pl.pallas_call(
        _kernel,
        in_specs=[anyspec] * 7,
        out_specs=anyspec,
        out_shape=jax.ShapeDtypeStruct((S, D), BF),
        scratch_shapes=[
            pltpu.VMEM((S, D), BF),
            pltpu.VMEM((D, 3 * D), BF),
            pltpu.VMEM((DH, DH, H), BF),
            pltpu.VMEM((D, D), BF),
            pltpu.VMEM((D, F), BF),
            pltpu.VMEM((D, F), BF),
            pltpu.VMEM((F, D), BF),
            pltpu.VMEM((S, D), BF),
            pltpu.VMEM((S // 128, 8, 128), F32),
            pltpu.VMEM((NB, 128, TS), BF),
            pltpu.VMEM((2 * D, D), BF),
            pltpu.VMEM((D, D), BF),
            pltpu.VMEM((32, D), F32),
            pltpu.VMEM((NT3 - 1, 64, 128), BF),
            pltpu.VMEM((GW + 8, 2 * GW), BF),
            pltpu.SemaphoreType.DMA((14,)),
            pltpu.SemaphoreType.DMA((NB, sum(pc[3] for pc in PIECES))),
        ],
        compiler_params=pltpu.CompilerParams(vmem_limit_bytes=100 * 1024 * 1024,
                                             disable_semaphore_checks=True,
                                             disable_bounds_checks=True),
    )(A_x.reshape(S, D), A_wqkv, jnp.transpose(A_w_phi, (1, 2, 0)), A_wo, B_w1, B_w3, B_w2)
    return out.reshape(1, S, D)
```
